```python
import os as _os
_os.environ.setdefault("JAX_PLATFORMS", "cpu")
import jax
import jax.numpy as jnp

def _softmax(x, axis=-1):
    return jax.nn.softmax(x, axis=axis)
def _gelu(x):
    return jax.nn.gelu(x, approximate=True)
def _silu(x):
    return jax.nn.silu(x)
def _sigmoid(x):
    return jax.nn.sigmoid(x)
def _layernorm(x, axis=-1, eps=1e-5):
    m = jnp.mean(x, axis=axis, keepdims=True)
    v = jnp.var(x, axis=axis, keepdims=True)
    return (x - m) / jnp.sqrt(v + eps)
def _scatter_add(tgt, idx, src, axis=0):
    return tgt.at[idx].add(src)
def _segment_sum(src, seg, n):
    return jax.ops.segment_sum(src, seg, n)
class _Rng:
    def __init__(self, key):
        self._k = key
    def _next(self):
        self._k, sub = jax.random.split(self._k)
        return sub
    def normal(self, shape):
        return jax.random.normal(self._next(), shape, dtype=jnp.bfloat16)
    def randint(self, lo, hi, shape):
        return jax.random.randint(self._next(), shape, lo, hi, dtype=jnp.int32)
    def uniform(self, shape, lo=0.0, hi=1.0):
        return jax.random.uniform(self._next(), shape, jnp.bfloat16, lo, hi)
    def permutation(self, n):
        return jax.random.permutation(self._next(), n)


kernel_name = 'standalone__mha_softmax__near_ridge'

def setup_inputs():
    _rng = _Rng(jax.random.key(int.from_bytes(__import__("os").urandom(4), "little")))
    _w = (lambda a: (lambda t: t.astype(jnp.bfloat16) if jnp.issubdtype(t.dtype, jnp.floating) else t)(jnp.asarray(a)))
    B, H, Sq, Sk, D = 8, 32, 384, 512, 128
    return {
        "q": _w((lambda *s: _rng.normal(s) * 0.4)(B, H, Sq, D)),
        "k": _w((lambda *s: _rng.normal(s) * 0.4)(B, H, Sk, D)),
        "v": _w((lambda *s: _rng.normal(s) * 0.05)(B, H, Sk, D)),
    }

def reference(q, k, v):
    scale = q.shape[-1] ** -0.5
    scores = jnp.einsum("bhqd,bhkd->bhqk", q, k) * scale
    p = _softmax(scores, axis=-1)
    return jnp.einsum("bhqk,bhkd->bhqd", p, v)
```

```python
import functools, math
import jax
import jax.numpy as jnp
import jax.experimental.pallas as pl
import jax.experimental.pallas.tpu as pltpu

def _kernel(q_hbm, k_hbm, v_hbm, o_hbm, xb, ob, sem_in, sem_out, *, c, BH, G, NBC, PR, S, batches, Sq, Sk,
            RQ, RK, PAT, W, LEAD, P0, E, nowrite, nodma, SS_):
    nsteps = BH // G
    RING = NBC * G
    def start_head(h):
        slot = h % RING
        sem = sem_in.at[(h // G) % NBC]
        j = 0
        off = 0
        for (src, SS, R) in [(q_hbm, Sq, RQ), (k_hbm, Sk, RK), (v_hbm, Sk, RK)]:
            for r in range(0, SS, R):
                pltpu.make_async_copy(src.at[h, pl.ds(r, R)], xb.at[slot, pl.ds(off + r, R)], sem).start(priority=int(PAT[j % len(PAT)]))
                j += 1
            off += SS

    def wait_chunk(i):
        cs = i % NBC
        pltpu.make_async_copy(xb.at[pl.ds(cs * G, G)], xb.at[pl.ds(cs * G, G)], sem_in.at[cs]).wait()

    def write_batch(a0, a1):
        n = S // SS_
        def issue(t, carry):
            s = (t % n) * SS_ + t // n
            pltpu.make_async_copy(ob.at[pl.ds(a0, a1 - a0), pl.ds(s, 1)], o_hbm.at[pl.ds(a0, a1 - a0), pl.ds(s, 1)], sem_out).start()
            return carry
        jax.lax.fori_loop(0, S, issue, 0)

    npieces = Sq // PR
    HPA = S // npieces
    def compute(i):
        base = (i % NBC) * G
        for g in range(G):
            q = xb[base + g, 0:Sq]
            k = xb[base + g, Sq:Sq + Sk]
            v = xb[base + g, Sq + Sk:Sq + 2 * Sk]
            s = jax.lax.dot_general(q, k, (((1,), (1,)), ((), ())), preferred_element_type=jnp.float32)
            m = jnp.max(s, axis=-1, keepdims=True)
            p = jnp.exp2((s - m) * c)
            l = jnp.sum(p, axis=-1, keepdims=True)
            o = jnp.dot(p.astype(jnp.bfloat16), v, preferred_element_type=jnp.float32)
            r = pl.reciprocal(l, approx=True)
            r = r * (2.0 - l * r)
            o = (o * r).astype(ob.dtype)
            h = i * G + g
            a = h // HPA
            s0 = (h % HPA) * npieces
            for pi in range(npieces):
                ob[a, s0 + pi] = o[pi * PR:(pi + 1) * PR]

    nA = (BH - P0) // E
    assert P0 + nA * E == BH, (P0, nA, E)
    assert P0 + nA * (E - G) <= RING
    if not nodma:
        def pro(h, carry):
            start_head(h)
            return carry
        jax.lax.fori_loop(0, P0, pro, 0)

    def bodyA(i, carry):
        if not nodma:
            wait_chunk(i)
        compute(i)
        if not nodma:
            for e in range(E):
                start_head(P0 + i * E + e)
        return carry
    jax.lax.fori_loop(0, nA, bodyA, 0)

    assert W >= nA
    def bodyB(i, carry):
        if not nodma:
            @pl.when(jnp.logical_or(i < W, i >= nsteps - LEAD))
            def _():
                wait_chunk(i)
        @pl.when(i == W)
        def _():
            if not nodma:
                for j in range(W, nsteps - LEAD):
                    wait_chunk(j)
            if not nowrite:
                (it, a0, a1) = batches[0]
                assert a1 * HPA <= W * G
                write_batch(a0, a1)
        compute(i)
        if not nowrite:
            for (it, a0, a1) in batches[1:]:
                assert a1 * HPA <= (it + 1) * G
                if it < nsteps - 1:
                    @pl.when(i == it)
                    def _():
                        write_batch(a0, a1)
        return carry
    jax.lax.fori_loop(nA, nsteps, bodyB, 0)
    if not nowrite:
        for (it, a0, a1) in batches[1:]:
            if it >= nsteps - 1:
                write_batch(a0, a1)
        pltpu.make_async_copy(ob, o_hbm, sem_out).wait()
    else:
        cp = pltpu.make_async_copy(ob.at[pl.ds(0, 1)], o_hbm.at[pl.ds(0, 1)], sem_out); cp.start(); cp.wait()

def _build(G=4, NBC=16, PR=128, S=48, batches=None, RQ=128, RK=256, PAT="0101010", W=52, LEAD=0, P0=16, E=5, nowrite=False, nodma=False, dbc=True, SS_=16):
    @jax.jit
    def f(q, k, v):
        B, H, Sq, D = q.shape
        Sk = k.shape[2]
        BH = B * H
        c = (D ** -0.5) * math.log2(math.e)
        q3 = q.reshape(BH, Sq, D); k3 = k.reshape(BH, Sk, D); v3 = v.reshape(BH, Sk, D)
        A = BH * Sq // (S * PR)
        out = pl.pallas_call(
            functools.partial(_kernel, c=c, BH=BH, G=G, NBC=NBC, PR=PR, S=S, batches=batches, Sq=Sq, Sk=Sk,
                              RQ=RQ, RK=RK, PAT=PAT, W=W, LEAD=LEAD, P0=P0, E=E, nowrite=nowrite, nodma=nodma, SS_=SS_),
            in_specs=[pl.BlockSpec(memory_space=pl.ANY)] * 3,
            out_specs=pl.BlockSpec(memory_space=pl.ANY),
            out_shape=jax.ShapeDtypeStruct((A, S, PR, D), q.dtype),
            scratch_shapes=[pltpu.VMEM((NBC * G, Sq + 2 * Sk, D), q.dtype), pltpu.VMEM((A, S, PR, D), q.dtype),
                            pltpu.SemaphoreType.DMA((NBC,)), pltpu.SemaphoreType.DMA(())],
            compiler_params=pltpu.CompilerParams(vmem_limit_bytes=120*1024*1024, disable_bounds_checks=dbc),
        )(q3, k3, v3)
        return out.reshape(B, H, Sq, D)
    return f


_BATCHES = ((0, 0, 12), (59, 12, 15), (63, 15, 16))
pallas_standalone__mha_softmax__near_ridge_kernel = _build(batches=_BATCHES, W=50)
```

```python
import functools
import math

import jax
import jax.numpy as jnp
import jax.experimental.pallas as pl
import jax.experimental.pallas.tpu as pltpu

_G = 4
_NBC = 16
_E = 5
_P0 = 16
_W = 50
_UB = 2
_LH = 3
_PR = 128
_NS = 16
_NBLK = 3


def _read_plan(Sq, Sk):
    k_sizes = (176, 160, 176)
    assert sum(k_sizes) == Sk and Sq % 32 == 0
    plan, r = [], 0
    for n in k_sizes:
        plan.append((1, r, n, 0))
        plan.append((2, r, n, 1))
        r += n
    plan.append((0, 0, Sq // 2, 0))
    plan.append((0, Sq // 2, Sq // 2, 1))
    return tuple(plan)


def _kernel(q_hbm, k_hbm, v_hbm, o_hbm, xb, ob, sem_in, sem_out, *, c, BH, Sq, Sk,
            W, LH, UB, wb):
    G, NBC, E, P0, PR, NS, NBLK = _G, _NBC, _E, _P0, _PR, _NS, _NBLK
    nchunks = BH // G
    ring = NBC * G
    srcs = (q_hbm, k_hbm, v_hbm)
    offs = (0, Sq, Sq + Sk)
    plan = _read_plan(Sq, Sk)
    npieces = Sq // PR
    hpa = NS * NBLK // npieces
    nblocks = BH // hpa

    def start_head(h):
        slot = h % ring
        si = jnp.where(h >= BH - LH, NBC, (h // G) % NBC)
        for (a, r0, n, prio) in plan:
            pltpu.make_async_copy(
                srcs[a].at[h, pl.ds(r0, n)],
                xb.at[slot, pl.ds(offs[a] + r0, n)],
                sem_in.at[si],
            ).start(priority=prio)

    def wait_heads(h0, n, si):
        dst = xb.at[pl.ds(h0 % ring, n)]
        pltpu.make_async_copy(dst, dst, sem_in.at[si]).wait()

    def wait_chunk(i, n=G):
        wait_heads(i * G, n, i % NBC)

    def write_wide(a0, a1):
        def issue(t, carry):
            b, s = t % NBLK, t // NBLK
            pltpu.make_async_copy(ob.at[pl.ds(a0, a1 - a0), b, s],
                                  o_hbm.at[pl.ds(a0, a1 - a0), b, s], sem_out).start()
            return carry
        jax.lax.fori_loop(0, NBLK * NS, issue, 0)

    def write_narrow(a0, a1):
        def issue(s, carry):
            pltpu.make_async_copy(ob.at[pl.ds(a0, a1 - a0), :, s],
                                  o_hbm.at[pl.ds(a0, a1 - a0), :, s], sem_out).start()
            return carry
        jax.lax.fori_loop(0, NS, issue, 0)

    def compute(i):
        base = (i % NBC) * G
        for g in range(G):
            q = xb[base + g, 0:Sq]
            k = xb[base + g, Sq:Sq + Sk]
            v = xb[base + g, Sq + Sk:Sq + 2 * Sk]
            s = jax.lax.dot_general(q, k, (((1,), (1,)), ((), ())),
                                    preferred_element_type=jnp.float32)
            m = jnp.max(s, axis=-1, keepdims=True)
            p = jnp.exp2((s - m) * c)
            l = jnp.sum(p, axis=-1, keepdims=True)
            o = jnp.dot(p.astype(v.dtype), v, preferred_element_type=jnp.float32)
            r = pl.reciprocal(l, approx=True)
            r = r * (2.0 - l * r)
            o = (o * r).astype(ob.dtype)
            h = i * G + g
            a = h // hpa
            j0 = (h % hpa) * npieces
            for pi in range(npieces):
                j = j0 + pi
                ob[a, j // NS, j % NS] = o[pi * PR:(pi + 1) * PR]

    nA = (BH - P0) // E
    assert P0 + nA * E == BH
    assert P0 + nA * (E - G) <= ring
    assert nA <= W and (W - nA) % UB == 0 and (nchunks - W) % UB == 0 and 0 < LH <= G

    def prologue(h, carry):
        start_head(h)
        return carry
    jax.lax.fori_loop(0, P0, prologue, 0)

    def body_a(i, carry):
        wait_chunk(i)
        compute(i)
        for e in range(E):
            start_head(P0 + i * E + e)
        return carry
    jax.lax.fori_loop(0, nA, body_a, 0)

    wb1, wb2_it, wb2 = wb
    assert wb1 * hpa <= W * G and wb2 * hpa <= (wb2_it + 1) * G and (wb2_it + 1) % UB == 0

    def body_b(ii, carry):
        i0 = ii * UB

        @pl.when(i0 < W)
        def _():
            for u in range(UB):
                wait_chunk(i0 + u)

        @pl.when(i0 == W)
        def _():
            for j in range(W, nchunks - 1):
                wait_chunk(j)
            if LH < G:
                wait_chunk(nchunks - 1, G - LH)
            write_wide(0, wb1)

        @pl.when(i0 + UB == nchunks)
        def _():
            wait_heads(BH - LH, LH, NBC)

        for u in range(UB):
            compute(i0 + u)

        @pl.when(i0 + UB - 1 == wb2_it)
        def _():
            write_narrow(wb1, wb2)
        return carry
    jax.lax.fori_loop(nA // UB, nchunks // UB, body_b, 0)

    write_narrow(wb2, nblocks)
    pltpu.make_async_copy(ob, o_hbm, sem_out).wait()


def build(W=_W, LH=_LH, UB=_UB, wb=(12, 59, 15)):
    @jax.jit
    def f(q, k, v):
        B, H, Sq, D = q.shape
        Sk = k.shape[2]
        BH = B * H
        c = (D ** -0.5) * math.log2(math.e)
        hpa = _NS * _NBLK * _PR // Sq
        oshape = (BH // hpa, _NBLK, _NS, _PR, D)
        out = pl.pallas_call(
            functools.partial(_kernel, c=c, BH=BH, Sq=Sq, Sk=Sk, W=W, LH=LH, UB=UB, wb=wb),
            in_specs=[pl.BlockSpec(memory_space=pl.ANY)] * 3,
            out_specs=pl.BlockSpec(memory_space=pl.ANY),
            out_shape=jax.ShapeDtypeStruct(oshape, q.dtype),
            scratch_shapes=[
                pltpu.VMEM((_NBC * _G, Sq + 2 * Sk, D), q.dtype),
                pltpu.VMEM(oshape, q.dtype),
                pltpu.SemaphoreType.DMA((_NBC + 1,)),
                pltpu.SemaphoreType.DMA(()),
            ],
            compiler_params=pltpu.CompilerParams(
                vmem_limit_bytes=100 * 1024 * 1024, disable_bounds_checks=True),
        )(q.reshape(BH, Sq, D), k.reshape(BH, Sk, D), v.reshape(BH, Sk, D))
        return out.reshape(B, H, Sq, D)
    return f

pallas_standalone__mha_softmax__near_ridge_kernel = build()
```

```python
import functools
import math

import jax
import jax.numpy as jnp
import jax.experimental.pallas as pl
import jax.experimental.pallas.tpu as pltpu

_G = 4
_NBC = 16
_E = 5
_P0 = 16
_UA = 2
_UB = 2
_W = 50
_LH = 3
_PR = 128
_NS = 16
_NBLK = 3
_WB1 = 12
_WB2 = 15
_WB2_AT = 59


def _read_plan(sq, sk):
    a = (sk // 3 + 15) // 16 * 16
    plan, r = [], 0
    for n in (a, sk - 2 * a, a):
        plan.append((1, r, n, 0))
        plan.append((2, r, n, 1))
        r += n
    plan.append((0, 0, sq // 2, 0))
    plan.append((0, sq // 2, sq // 2, 1))
    return tuple(plan)


def _kernel(q_hbm, k_hbm, v_hbm, o_hbm, xb, ob, sem_in, sem_out, *, c, bh, sq, sk):
    nchunks = bh // _G
    ring = _NBC * _G
    srcs = (q_hbm, k_hbm, v_hbm)
    offs = (0, sq, sq + sk)
    plan = _read_plan(sq, sk)
    npieces = sq // _PR
    hpb = _NS * _NBLK // npieces
    nblocks = bh // hpb
    n_a = (bh - _P0) // _E

    assert _P0 + n_a * _E == bh and _P0 + n_a * (_E - _G) <= ring
    assert n_a % _UA == 0 and n_a % _UB == 0 and n_a <= _W
    assert _W % _UB == 0 and nchunks % _UB == 0 and 0 < _LH < _G
    assert _WB1 * hpb <= _W * _G and _WB2 * hpb <= (_WB2_AT + 1) * _G
    assert (_WB2_AT + 1) % _UB == 0 and _W <= _WB2_AT < nchunks - 1

    def start_head(h):
        slot = h % ring
        si = jnp.where(h >= bh - _LH, _NBC, (h // _G) % _NBC)
        for (a, r0, n, prio) in plan:
            pltpu.make_async_copy(
                srcs[a].at[h, pl.ds(r0, n)],
                xb.at[slot, pl.ds(offs[a] + r0, n)],
                sem_in.at[si],
            ).start(priority=prio)

    def wait_heads(h0, n, si):
        dst = xb.at[pl.ds(h0 % ring, n)]
        pltpu.make_async_copy(dst, dst, sem_in.at[si]).wait()

    def wait_chunk(i, n=_G):
        wait_heads(i * _G, n, i % _NBC)

    def write_wide(a0, a1):
        def issue(t, carry):
            b, s = t % _NBLK, t // _NBLK
            pltpu.make_async_copy(ob.at[pl.ds(a0, a1 - a0), b, s],
                                  o_hbm.at[pl.ds(a0, a1 - a0), b, s], sem_out).start()
            return carry
        jax.lax.fori_loop(0, _NBLK * _NS, issue, 0)

    def write_narrow(a0, a1):
        def issue(s, carry):
            pltpu.make_async_copy(ob.at[pl.ds(a0, a1 - a0), :, s],
                                  o_hbm.at[pl.ds(a0, a1 - a0), :, s], sem_out).start()
            return carry
        jax.lax.fori_loop(0, _NS, issue, 0)

    def compute(i):
        base = (i % _NBC) * _G
        for g in range(_G):
            q = xb[base + g, 0:sq]
            k = xb[base + g, sq:sq + sk]
            v = xb[base + g, sq + sk:sq + 2 * sk]
            s = jax.lax.dot_general(q, k, (((1,), (1,)), ((), ())),
                                    preferred_element_type=jnp.float32)
            m = jnp.max(s, axis=-1, keepdims=True)
            p = jnp.exp2((s - m) * c)
            l = jnp.sum(p, axis=-1, keepdims=True)
            o = jnp.dot(p.astype(v.dtype), v, preferred_element_type=jnp.float32)
            r = pl.reciprocal(l, approx=True)
            r = r * (2.0 - l * r)
            o = (o * r).astype(ob.dtype)
            h = i * _G + g
            a = h // hpb
            j0 = (h % hpb) * npieces
            for pi in range(npieces):
                j = j0 + pi
                ob[a, j // _NS, j % _NS] = o[pi * _PR:(pi + 1) * _PR]

    def prologue(h, carry):
        start_head(h)
        return carry
    jax.lax.fori_loop(0, _P0, prologue, 0)

    def body_a(ii, carry):
        for u in range(_UA):
            i = ii * _UA + u
            wait_chunk(i)
            compute(i)
            for e in range(_E):
                start_head(_P0 + i * _E + e)
        return carry
    jax.lax.fori_loop(0, n_a // _UA, body_a, 0)

    def body_b(ii, carry):
        i0 = ii * _UB

        @pl.when(i0 < _W)
        def _():
            for u in range(_UB):
                wait_chunk(i0 + u)

        @pl.when(i0 == _W)
        def _():
            for j in range(_W, nchunks - 1):
                wait_chunk(j)
            wait_chunk(nchunks - 1, _G - _LH)
            write_wide(0, _WB1)

        @pl.when(i0 + _UB == nchunks)
        def _():
            wait_heads(bh - _LH, _LH, _NBC)

        for u in range(_UB):
            compute(i0 + u)

        @pl.when(i0 + _UB - 1 == _WB2_AT)
        def _():
            write_narrow(_WB1, _WB2)
        return carry
    jax.lax.fori_loop(n_a // _UB, nchunks // _UB, body_b, 0)

    write_narrow(_WB2, nblocks)
    pltpu.make_async_copy(ob, o_hbm, sem_out).wait()


@jax.jit
def pallas_standalone__mha_softmax__near_ridge_kernel(
    q: jax.Array,
    k: jax.Array,
    v: jax.Array,
):
    B, H, Sq, D = q.shape
    Sk = k.shape[2]
    BH = B * H
    c = (D ** -0.5) * math.log2(math.e)
    hpb = _NS * _NBLK * _PR // Sq
    o_shape = (BH // hpb, _NBLK, _NS, _PR, D)
    out = pl.pallas_call(
        functools.partial(_kernel, c=c, bh=BH, sq=Sq, sk=Sk),
        in_specs=[pl.BlockSpec(memory_space=pl.ANY)] * 3,
        out_specs=pl.BlockSpec(memory_space=pl.ANY),
        out_shape=jax.ShapeDtypeStruct(o_shape, q.dtype),
        scratch_shapes=[
            pltpu.VMEM((_NBC * _G, Sq + 2 * Sk, D), q.dtype),
            pltpu.VMEM(o_shape, q.dtype),
            pltpu.SemaphoreType.DMA((_NBC + 1,)),
            pltpu.SemaphoreType.DMA(()),
        ],
        compiler_params=pltpu.CompilerParams(
            vmem_limit_bytes=100 * 1024 * 1024,
            disable_bounds_checks=True,
        ),
    )(q.reshape(BH, Sq, D), k.reshape(BH, Sk, D), v.reshape(BH, Sk, D))
    return out.reshape(B, H, Sq, D)
```

```python
import functools
import math

import jax
import jax.numpy as jnp
import jax.experimental.pallas as pl
import jax.experimental.pallas.tpu as pltpu

_G = 4
_NBC = 16
_E = 5
_P0 = 16
_W = 49
_UB = 2
_LH = 3
_PR = 128
_NS = 16
_NBLK = 3
_WB1 = 12
_TRIG = ((56, 12, 14), (60, 14, 15))
_READS = ((2, 96, 0), (1, 112, 1), (0, 96, 0), (2, 256, 1), (1, 240, 0),
          (0, 144, 1), (2, 160, 0), (0, 144, 0), (1, 160, 1))


def _div(x, n):
    assert n & (n - 1) == 0
    if isinstance(x, int):
        return x // n
    return jax.lax.shift_right_logical(x, n.bit_length() - 1)


def _mod(x, n):
    assert n & (n - 1) == 0
    if isinstance(x, int):
        return x % n
    return jax.lax.bitwise_and(x, n - 1)


def _kernel(q_hbm, k_hbm, v_hbm, o_hbm, xb, ob, sem_in, sem_out, *, c, bh, sq, sk):
    nchunks = bh // _G
    ring = _NBC * _G
    srcs = (q_hbm, k_hbm, v_hbm)
    offs = (0, sq, sq + sk)
    npieces = sq // _PR
    hpb = _NS * _NBLK // npieces
    nblocks = bh // hpb
    n_a = (bh - _P0) // _E
    n_b = (nchunks - 1 - _W) // _UB

    plan, done = [], [0, 0, 0]
    for (a, n, prio) in _READS:
        plan.append((a, done[a], n, prio))
        done[a] += n
    assert done == [sq, sk, sk]

    assert _P0 + n_a * _E == bh and _P0 >= _G and _E >= _G
    assert _P0 + n_a * (_E - _G) <= ring
    assert n_a <= _W and _W + n_b * _UB == nchunks - 1 and 0 < _LH < _G
    assert _WB1 * hpb <= _W * _G and _TRIG[0][1] == _WB1 and _TRIG[-1][2] == nblocks - 1
    for t, (at, a0, a1) in enumerate(_TRIG):
        assert a1 * hpb <= (at + 1) * _G and (at + 1 - _W) % _UB == 0 and _W <= at
        assert t == 0 or a0 == _TRIG[t - 1][2]

    def start_head(h):
        slot = _mod(h, ring)
        si = jnp.where(h >= bh - _LH, _NBC, _mod(_div(h, _G), _NBC))
        for (a, r0, n, prio) in plan:
            pltpu.make_async_copy(
                srcs[a].at[h, pl.ds(r0, n)],
                xb.at[slot, pl.ds(offs[a] + r0, n)],
                sem_in.at[si],
            ).start(priority=prio)

    def wait_heads(h0, n, si):
        dst = xb.at[pl.ds(_mod(h0, ring), n)]
        pltpu.make_async_copy(dst, dst, sem_in.at[si]).wait()

    def wait_chunk(i, n=_G):
        wait_heads(i * _G, n, _mod(i, _NBC))

    def write(idx):
        pltpu.make_async_copy(ob.at[idx], o_hbm.at[idx], sem_out).start()

    def write_wide(a0, a1):
        def issue(s, carry):
            for b in range(_NBLK):
                write((pl.ds(a0, a1 - a0), b, s))
            return carry
        jax.lax.fori_loop(0, _NS, issue, 0)

    def write_narrow(a0, a1):
        def issue(s, carry):
            write((pl.ds(a0, a1 - a0), slice(None), s))
            return carry
        jax.lax.fori_loop(0, _NS, issue, 0)

    def write_range(a, j0, j1):
        for s in range(_NS):
            bs = [b for b in range(_NBLK) if j0 <= b * _NS + s < j1]
            if bs:
                write((a, pl.ds(bs[0], len(bs)), s))

    def compute(i):
        base = _mod(i, _NBC) * _G
        for g in range(_G):
            q = xb[base + g, 0:sq]
            k = xb[base + g, sq:sq + sk]
            v = xb[base + g, sq + sk:sq + 2 * sk]
            s = jax.lax.dot_general(q, k, (((1,), (1,)), ((), ())),
                                    preferred_element_type=jnp.float32)
            m = jnp.max(s, axis=-1, keepdims=True)
            p = jnp.exp2((s - m) * c)
            l = jnp.sum(p, axis=-1, keepdims=True)
            o = jnp.dot(p.astype(v.dtype), v, preferred_element_type=jnp.float32)
            r = pl.reciprocal(l, approx=True)
            r = r * (2.0 - l * r)
            o = (o * r).astype(ob.dtype)
            h = i * _G + g
            a = _div(h, hpb)
            j0 = _mod(h, hpb) * npieces
            for pi in range(npieces):
                j = j0 + pi
                ob[a, _div(j, _NS), _mod(j, _NS)] = o[pi * _PR:(pi + 1) * _PR]

    def prologue(h, carry):
        start_head(h)
        return carry
    jax.lax.fori_loop(0, _P0, prologue, 0)

    def body_a(i, carry):
        wait_chunk(i)
        compute(i)
        for e in range(_E):
            start_head(_P0 + i * _E + e)
        return carry
    jax.lax.fori_loop(0, n_a, body_a, 0)

    for i in range(n_a, _W):
        wait_chunk(i)
        compute(i)
    for i in range(_W, nchunks - 1):
        wait_chunk(i)
    wait_chunk(nchunks - 1, _G - _LH)
    write_wide(0, _WB1)

    tail = (hpb - _G) * npieces
    def body_b(ii, carry):
        i0 = _W + ii * _UB
        for u in range(_UB):
            compute(i0 + u)
        last = i0 + _UB - 1
        for (at, a0, a1) in _TRIG:
            @pl.when(last == at)
            def _():
                write_narrow(a0, a1)

        @pl.when(last == nchunks - 2)
        def _():
            write_range(nblocks - 1, 0, tail)
        return carry
    jax.lax.fori_loop(0, n_b, body_b, 0)

    wait_heads(bh - _LH, _LH, _NBC)
    compute(nchunks - 1)
    write_range(nblocks - 1, tail, hpb * npieces)
    pltpu.make_async_copy(ob, o_hbm, sem_out).wait()


@jax.jit
def pallas_standalone__mha_softmax__near_ridge_kernel(
    q: jax.Array,
    k: jax.Array,
    v: jax.Array,
):
    B, H, Sq, D = q.shape
    Sk = k.shape[2]
    BH = B * H
    c = (D ** -0.5) * math.log2(math.e)
    hpb = _NS * _NBLK * _PR // Sq
    o_shape = (BH // hpb, _NBLK, _NS, _PR, D)
    out = pl.pallas_call(
        functools.partial(_kernel, c=c, bh=BH, sq=Sq, sk=Sk),
        in_specs=[pl.BlockSpec(memory_space=pl.ANY)] * 3,
        out_specs=pl.BlockSpec(memory_space=pl.ANY),
        out_shape=jax.ShapeDtypeStruct(o_shape, q.dtype),
        scratch_shapes=[
            pltpu.VMEM((_NBC * _G, Sq + 2 * Sk, D), q.dtype),
            pltpu.VMEM(o_shape, q.dtype),
            pltpu.SemaphoreType.DMA((_NBC + 1,)),
            pltpu.SemaphoreType.DMA(()),
        ],
        compiler_params=pltpu.CompilerParams(
            vmem_limit_bytes=100 * 1024 * 1024,
            disable_bounds_checks=True,
        ),
    )(q.reshape(BH, Sq, D), k.reshape(BH, Sk, D), v.reshape(BH, Sk, D))
    return out.reshape(B, H, Sq, D)
```
